```python
import os as _os
_os.environ.setdefault("JAX_PLATFORMS", "cpu")
import jax
import jax.numpy as jnp

def _softmax(x, axis=-1):
    return jax.nn.softmax(x, axis=axis)
def _gelu(x):
    return jax.nn.gelu(x, approximate=True)
def _silu(x):
    return jax.nn.silu(x)
def _sigmoid(x):
    return jax.nn.sigmoid(x)
def _layernorm(x, axis=-1, eps=1e-5):
    m = jnp.mean(x, axis=axis, keepdims=True)
    v = jnp.var(x, axis=axis, keepdims=True)
    return (x - m) / jnp.sqrt(v + eps)
def _scatter_add(tgt, idx, src, axis=0):
    return tgt.at[idx].add(src)
def _segment_sum(src, seg, n):
    return jax.ops.segment_sum(src, seg, n)
class _Rng:
    def __init__(self, key):
        self._k = key
    def _next(self):
        self._k, sub = jax.random.split(self._k)
        return sub
    def normal(self, shape):
        return jax.random.normal(self._next(), shape, dtype=jnp.bfloat16)
    def randint(self, lo, hi, shape):
        return jax.random.randint(self._next(), shape, lo, hi, dtype=jnp.int32)
    def uniform(self, shape, lo=0.0, hi=1.0):
        return jax.random.uniform(self._next(), shape, jnp.bfloat16, lo, hi)
    def permutation(self, n):
        return jax.random.permutation(self._next(), n)


kernel_name = 'standalone__gqa_block_cached__near_ridge'

def setup_inputs():
    _rng = _Rng(jax.random.key(int.from_bytes(__import__("os").urandom(4), "little")))
    _w = (lambda a: (lambda t: t.astype(jnp.bfloat16) if jnp.issubdtype(t.dtype, jnp.floating) else t)(jnp.asarray(a)))
    B, Sq, D = 8, 80, 512
    Hq, Hkv, Sk, Dh = 32, 8, 2048, 128
    assert Hq % Hkv == 0, (Hq, Hkv)
    return {
        "x": _w((lambda *s: _rng.normal(s) * 0.8)(B, Sq, D)),
        "k_cache": _w((lambda *s: _rng.normal(s) * 0.8)(B, Hkv, Sk, Dh)),
        "v_cache": _w((lambda *s: _rng.normal(s) * 0.05)(B, Hkv, Sk, Dh)),
        "wq": _w((lambda *s: _rng.normal(s) * 0.8)(D, Hq * Dh) * (D ** -0.5)),
        "wo": _w((lambda *s: _rng.normal(s) * 0.05)(Hq * Dh, D) * ((Hq * Dh) ** -0.5)),
    }

def reference(x, k_cache, v_cache, wq, wo):
    B, Sq, D = x.shape
    Hq, Dh = 32, 128
    Hkv = k_cache.shape[1]
    rep = Hq // Hkv
    q = (lambda x, *d: x.transpose(*d))((x @ wq).reshape(B, Sq, Hq, Dh), 0, 2, 1, 3)
    k = jnp.repeat(k_cache, rep, axis=1)
    v = jnp.repeat(v_cache, rep, axis=1)
    scores = jnp.einsum("bhqd,bhkd->bhqk", q, k) * (Dh ** -0.5)
    p = _softmax(scores, axis=-1)
    o = jnp.einsum("bhqk,bhkd->bhqd", p, v)
    return (lambda x, *d: x.transpose(*d))(o, 0, 2, 1, 3).reshape(B, Sq, Hq * Dh) @ wo
```

```python
import functools
import jax
import jax.numpy as jnp
import numpy as np
from jax.experimental import pallas as pl
from jax.experimental.pallas import tpu as pltpu

LOG2E = 1.4426950408889634
NT = (((1,), (1,)), ((), ()))
NN = (((1,), (0,)), ((), ()))


def _lane_tiles(a):
    return [a[:, i * 128:(i + 1) * 128] for i in range(a.shape[1] // 128)]


def _tree(op, xs):
    while len(xs) > 1:
        xs = [op(xs[i], xs[i + 1]) if i + 1 < len(xs) else xs[i] for i in range(0, len(xs), 2)]
    return xs[0]


def _kernel(x_hbm, k_hbm, v_hbm, wq_hbm, wo_hbm, out_hbm,
            x_buf, wq_buf, wo_buf, k_buf, v_buf, out_buf, acc_scrs, s_scrs,
            x_sem, wq_sem, wo_sem, k_sem, k0_sem, v_sem, out_sem,
            *, B, Sq, Sk, rep, Dh, Hkv, ck, cv, qlead, olag, tie2, depth, xgroups, order, kpin, vpin, k0split):
    scale = (Dh ** -0.5) * LOG2E
    G = rep * Dh
    bf = jnp.bfloat16
    NK = Sk // ck

    def k_copy(h, b):
        return pltpu.make_async_copy(k_hbm.at[b, h], k_buf.at[b], k_sem.at[b])

    def k0_copy(j):
        return pltpu.make_async_copy(k_hbm.at[0, 0, j * ck:(j + 1) * ck], k_buf.at[0, j * ck:(j + 1) * ck], k0_sem.at[j])

    def v_copy(h, b):
        return pltpu.make_async_copy(v_hbm.at[b, h], v_buf.at[b], v_sem.at[b])

    def wq_copy(h):
        return pltpu.make_async_copy(wq_hbm.at[:, pl.ds(pl.multiple_of(h * G, G), G)], wq_buf.at[h % 2], wq_sem.at[h % 2])

    def wo_copy(h):
        return pltpu.make_async_copy(wo_hbm.at[pl.ds(pl.multiple_of(h * G, G), G), :], wo_buf.at[h % 2], wo_sem.at[h % 2])

    def x_copy(g):
        lo, hi = xgroups[g] * Sq, xgroups[g + 1] * Sq
        return pltpu.make_async_copy(x_hbm.at[lo:hi], x_buf.at[lo:hi], x_sem.at[g])

    def out_copy(b):
        return pltpu.make_async_copy(out_buf.at[b], out_hbm.at[b], out_sem.at[b])

    def pin(spare_ref, value):
        spare_ref[...] = value[0:16, 0:128].astype(bf)

    first = []
    for tok in order.split():
        kind, idx = tok[0], int(tok[1:])
        if kind == "k" and idx == 0 and k0split:
            first += [k0_copy(j) for j in range(NK)]
        else:
            first.append({"q": wq_copy, "o": wo_copy, "x": x_copy, "k": lambda i: k_copy(0, i), "v": lambda i: v_copy(0, i)}[kind](idx))

    def issue(i, c):
        for n, cp in enumerate(first):
            pl.when(i == n)(cp.start)
        return c

    jax.lax.fori_loop(0, len(first), issue, 0)
    for b in range(B):
        acc_scrs[b][...] = jnp.zeros_like(acc_scrs[b])

    def body(h, carry):
        par = h % 2

        def prefetch(b):
            nb = b + depth
            if nb < B:
                k_copy(h, nb).start()
                v_copy(h, nb).start()
            else:
                @pl.when(h + 1 < Hkv)
                def _():
                    if nb == B:
                        wq_copy(h + 1).start()
                    k_copy(h + 1, nb - B).start()
                    if nb == B + 1:
                        wo_copy(h + 1).start()
                    v_copy(h + 1, nb - B).start()

        def Q(b, after):
            if b in xgroups[:-1]:
                if after is not None:
                    pin(x_buf.at[B * Sq:B * Sq + 16, 0:128], after)

                @pl.when(h == 0)
                def _():
                    x_copy(xgroups.index(b)).wait()
            q = jax.lax.dot_general(x_buf[b * Sq:(b + 1) * Sq, :], wq_buf[par], NN, preferred_element_type=jnp.float32) * scale
            return jnp.concatenate([q[:, r * Dh:(r + 1) * Dh] for r in range(rep)], axis=0).astype(bf), q

        def QK(b, q, after):
            pin(k_buf.at[B, 0:16, :], after)
            if b == 0 and k0split:
                pl.when(h > 0)(k_copy(h, b).wait)
            else:
                k_copy(h, b).wait()
            m_run = None
            ss = []
            for j in range(NK):
                if b == 0 and k0split:
                    if j >= 2:
                        pin(k_buf.at[B, 0:16, :], ss[j - 2])
                    pl.when(h == 0)(k0_copy(j).wait)
                s = jax.lax.dot_general(q, k_buf[b, j * ck:(j + 1) * ck, :], NT, preferred_element_type=jnp.float32)
                ss.append(s)
                s_scrs[b % 2][:, j * ck:(j + 1) * ck] = s
                mp = _tree(jnp.maximum, _lane_tiles(s))
                m_run = mp if m_run is None else jnp.maximum(m_run, mp)
            return jnp.max(m_run, axis=-1, keepdims=True), ss

        def PV(b, m, after):
            pin(v_buf.at[B, 0:16, :], after)
            v_copy(h, b).wait()
            s = s_scrs[b % 2]
            nl = o_run = None
            parts = []
            for j in range(Sk // cv):
                p = jnp.exp2(s[:, j * cv:(j + 1) * cv] - m)
                pt = _lane_tiles(p)
                lp = _tree(jnp.add, pt)
                nl = -lp if nl is None else nl - lp
                pt[0] = jnp.maximum(pt[0], nl)
                p = jnp.concatenate(pt, axis=1)
                o = jax.lax.dot_general(p.astype(bf), v_buf[b, j * cv:(j + 1) * cv, :], NN, preferred_element_type=jnp.float32)
                parts.append(o)
                o_run = o if o_run is None else o_run + o
            if tie2 == 1 or (tie2 == 2 and b == B - 1):
                nl = jnp.minimum(nl, jnp.abs(o_run))
            l = jnp.sum(nl, axis=-1, keepdims=True)
            o = o_run * (-1.0 / l)
            return jnp.concatenate([o[r * Sq:(r + 1) * Sq, :] for r in range(rep)], axis=1).astype(bf), parts

        def O(b, o, after):
            if b == 0:
                pin(wo_buf.at[2, 0:16, 0:128], after)
                wo_copy(h).wait()
            part = jax.lax.dot_general(o, wo_buf[par], NN, preferred_element_type=jnp.float32)
            acc = acc_scrs[b][...] + part
            acc_scrs[b][...] = acc
            out_buf[b] = acc.astype(out_buf.dtype)

            @pl.when(h == Hkv - 1)
            def _():
                out_copy(b).start()

        qs, os_ = {}, {}
        wq_copy(h).wait()
        raw = []
        for b in range(qlead):
            qs[b], qf = Q(b, raw[b - 2] if b >= 2 else None)
            raw.append(qf)
        kafter = raw[max(qlead - 2, 0)]
        for b in range(B):
            m, ss = QK(b, qs[b], kafter)
            prefetch(b)
            if b + qlead < B:
                qs[b + qlead], _ = Q(b + qlead, ss[NK - 2])
            if b - olag >= 0:
                O(b - olag, os_[b - olag], ss[NK - 2])
            os_[b], parts = PV(b, m, ss[NK - vpin])
            kafter = parts[len(parts) - kpin]
        for b in range(B - olag, B):
            O(b, os_[b], None)
        return carry

    jax.lax.fori_loop(0, Hkv, body, 0)
    for b in range(B):
        out_copy(b).wait()


@jax.jit
def pallas_standalone__gqa_block_cached__near_ridge_kernel(x, k_cache, v_cache, wq, wo):
    B, Sq, D = x.shape
    _, Hkv, Sk, Dh = k_cache.shape
    rep = wq.shape[1] // Dh // Hkv
    bf = jnp.bfloat16
    ck, xg = 512, (0, 1, 2, 3, 8)
    return pl.pallas_call(
        functools.partial(_kernel, B=B, Sq=Sq, Sk=Sk, rep=rep, Dh=Dh, Hkv=Hkv, ck=ck, cv=256, qlead=2, olag=2,
                          tie2=2, depth=4, xgroups=xg, order="q0 x0 x1 k0 x2 v0 k1 x3 v1 k2 o0 v2 k3 v3",
                          kpin=3, vpin=1, k0split=1),
        in_specs=[pl.BlockSpec(memory_space=pl.ANY)] * 5,
        out_specs=pl.BlockSpec(memory_space=pl.ANY),
        out_shape=jax.ShapeDtypeStruct((B, Sq, D), x.dtype),
        scratch_shapes=[
            pltpu.VMEM((B * Sq + 16, D), bf),
            pltpu.VMEM((3, D, rep * Dh), bf),
            pltpu.VMEM((3, rep * Dh, D), bf),
            pltpu.VMEM((B + 1, Sk, Dh), bf),
            pltpu.VMEM((B + 1, Sk, Dh), bf),
            pltpu.VMEM((B, Sq, D), bf),
            [pltpu.VMEM((Sq, D), jnp.float32) for _ in range(B)],
            [pltpu.VMEM((rep * Sq, Sk), jnp.float32) for _ in range(2)],
            pltpu.SemaphoreType.DMA((len(xg) - 1,)),
            pltpu.SemaphoreType.DMA((2,)),
            pltpu.SemaphoreType.DMA((2,)),
            pltpu.SemaphoreType.DMA((B,)),
            pltpu.SemaphoreType.DMA((Sk // ck,)),
            pltpu.SemaphoreType.DMA((B,)),
            pltpu.SemaphoreType.DMA((B,)),
        ],
        compiler_params=pltpu.CompilerParams(
            vmem_limit_bytes=100 * 1024 * 1024,
            flags={"XLA_TPU_RESCHEDULE_DMA_DONES": True},
            disable_bounds_checks=True,
        ),
    )(x.reshape(B * Sq, D), k_cache, v_cache, wq, wo)
```

```python
import functools

import jax
import jax.numpy as jnp
from jax.experimental import pallas as pl
from jax.experimental.pallas import tpu as pltpu

_LOG2E = 1.4426950408889634
_NN = (((1,), (0,)), ((), ()))
_NT = (((1,), (1,)), ((), ()))
_LANES = 128

_QK_KEYS = 256
_PV_KEYS = 128
_DEPTH = 4
_COLD = 3
_CHUNKS = 4
_FIRST_LOADS = "q0 x0 k0 x1 v0 k1 x2 o0 v1 k2 x3 v2 k3 x4 x5 x6 x7 v3".split()


def _dot(a, b, dims=_NN):
    return jax.lax.dot_general(a, b, dims, preferred_element_type=jnp.float32)


def _lane_tiles(a):
    return [a[:, i:i + _LANES] for i in range(0, a.shape[1], _LANES)]


def _kernel(x_hbm, k_hbm, v_hbm, wq_hbm, wo_hbm, out_hbm,
            x_buf, wq_buf, wo_buf, k_buf, v_buf, out_buf, acc_bufs, s_bufs, in_sems, out_sems,
            *, rep):
    B, Sq, _ = x_hbm.shape
    _, Hkv, Sk, Dh = k_hbm.shape
    G = rep * Dh
    bf16 = jnp.bfloat16
    chunk = Sk // _CHUNKS
    scale = (Dh ** -0.5) * _LOG2E

    sem_base, n_sems = {}, 0
    for name, count in (("wq", 2), ("wo", 2), ("x", B), ("k", B), ("v", B),
                        ("k_chunk", _COLD * _CHUNKS), ("v_chunk", _COLD * _CHUNKS)):
        sem_base[name] = n_sems
        n_sems += count

    def sem(name, i):
        return in_sems.at[sem_base[name] + i]

    kv = {"k": (k_hbm, k_buf), "v": (v_hbm, v_buf)}

    def kv_copy(kind, h, b):
        hbm, buf = kv[kind]
        return pltpu.make_async_copy(hbm.at[b, h], buf.at[b], sem(kind, b))

    def kv_chunk_copy(kind, b, j):
        hbm, buf = kv[kind]
        keys = slice(j * chunk, (j + 1) * chunk)
        return pltpu.make_async_copy(hbm.at[b, 0, keys], buf.at[b, keys],
                                     sem(kind + "_chunk", b * _CHUNKS + j))

    def wq_copy(h):
        cols = pl.ds(pl.multiple_of(h * G, G), G)
        return pltpu.make_async_copy(wq_hbm.at[:, cols], wq_buf.at[h & 1], sem("wq", h & 1))

    def wo_copy(h):
        rows = pl.ds(pl.multiple_of(h * G, G), G)
        return pltpu.make_async_copy(wo_hbm.at[rows, :], wo_buf.at[h & 1], sem("wo", h & 1))

    def x_copy(b):
        return pltpu.make_async_copy(x_hbm.at[b], x_buf.at[b], sem("x", b))

    def out_copy(b):
        return pltpu.make_async_copy(out_buf.at[b], out_hbm.at[b], out_sems.at[b])

    def hold_wait(spare, value):
        spare[...] = value[0:16, 0:_LANES].astype(bf16)

    for token in _FIRST_LOADS:
        kind, i = token[0], int(token[1:])
        if kind in kv and i < _COLD:
            for j in range(_CHUNKS):
                kv_chunk_copy(kind, i, j).start()
        elif kind in kv:
            kv_copy(kind, 0, i).start()
        else:
            {"q": wq_copy, "o": wo_copy, "x": x_copy}[kind](i).start()
    for acc in acc_bufs:
        acc[...] = jnp.zeros_like(acc)

    def head(h, carry):
        slot = h & 1

        def prefetch(b):
            nb = b + _DEPTH
            if nb < B:
                kv_copy("k", h, nb).start()
                kv_copy("v", h, nb).start()
            else:
                @pl.when(h + 1 < Hkv)
                def _():
                    if nb == B:
                        wq_copy(h + 1).start()
                    kv_copy("k", h + 1, nb - B).start()
                    if nb == B + 1:
                        wo_copy(h + 1).start()
                    kv_copy("v", h + 1, nb - B).start()

        def wait_kv(kind, b, key, after):
            if key == 0 or (b < _COLD and key % chunk == 0):
                if b <= _COLD:
                    hold_wait(kv[kind][1].at[B, 0:16, :], after)
                if b < _COLD:
                    if key == 0:
                        pl.when(h > 0)(kv_copy(kind, h, b).wait)
                    pl.when(h == 0)(kv_chunk_copy(kind, b, key // chunk).wait)
                else:
                    kv_copy(kind, h, b).wait()

        def q_proj(b, after):
            if after is not None and b <= _COLD:
                hold_wait(x_buf.at[B, 0:16, 0:_LANES], after)
            pl.when(h == 0)(x_copy(b).wait)
            q = _dot(x_buf[b], wq_buf[slot]) * scale
            stacked = jnp.concatenate([q[:, r * Dh:(r + 1) * Dh] for r in range(rep)], axis=0)
            return stacked.astype(bf16), q

        def scores(b, q, after):
            per_chunk = chunk // _QK_KEYS
            m, blocks = None, []
            for j, key in enumerate(range(0, Sk, _QK_KEYS)):
                keys = slice(key, key + _QK_KEYS)
                wait_kv("k", b, key, after if j == 0 else blocks[max(j - per_chunk, 0)])
                s = _dot(q, k_buf[b, keys, :], _NT)
                blocks.append(s)
                s_bufs[b % 2][:, keys] = s
                block_max = functools.reduce(jnp.maximum, _lane_tiles(s))
                m = block_max if m is None else jnp.maximum(m, block_max)
            return jnp.max(m, axis=-1, keepdims=True), blocks[-per_chunk]

        def attend(b, m, after):
            per_chunk = chunk // _PV_KEYS
            neg_l, o, blocks = None, None, []
            for j, key in enumerate(range(0, Sk, _PV_KEYS)):
                keys = slice(key, key + _PV_KEYS)
                wait_kv("v", b, key, after if j == 0 else blocks[max(j - per_chunk, 0)])
                p = _lane_tiles(jnp.exp2(s_bufs[b % 2][:, keys] - m))
                for tile in p:
                    neg_l = -tile if neg_l is None else neg_l - tile
                p[0] = jnp.maximum(p[0], neg_l)
                part = _dot(jnp.concatenate(p, axis=1).astype(bf16), v_buf[b, keys, :])
                blocks.append(part)
                o = part if o is None else o + part
            neg_l = jnp.minimum(neg_l, jnp.abs(o))
            l = -jnp.sum(neg_l, axis=-1, keepdims=True)
            return o * pl.reciprocal(l, full_range=False), blocks[-per_chunk]

        def out_proj(b, o, after):
            if b == 0:
                hold_wait(wo_buf.at[2, 0:16, 0:_LANES], after)
                wo_copy(h).wait()
            heads = [o[r * Sq:(r + 1) * Sq] for r in range(rep)]
            if b + 1 < B:
                part = _dot(jnp.concatenate(heads, axis=1).astype(bf16), wo_buf[slot])
                acc = acc_bufs[b][...] + part
            else:
                acc = acc_bufs[b][...]
                for r in range(rep):
                    part = _dot(heads[r].astype(bf16), wo_buf[slot, r * Dh:(r + 1) * Dh, :])
                    acc = acc + part
            acc_bufs[b][...] = acc
            out_buf[b] = acc.astype(out_buf.dtype)
            pl.when(h == Hkv - 1)(out_copy(b).start)
            return part

        wq_copy(h).wait()
        q, last = q_proj(0, None)
        o = None
        for b in range(B):
            m, last = scores(b, q, last)
            prefetch(b)
            if b + 1 < B:
                q, last = q_proj(b + 1, last)
            if b > 0:
                last = out_proj(b - 1, o, last)
            o, last = attend(b, m, last)
        out_proj(B - 1, o, None)
        return carry

    jax.lax.fori_loop(0, Hkv, head, 0)
    for b in range(B):
        out_copy(b).wait()


@jax.jit
def pallas_standalone__gqa_block_cached__near_ridge_kernel(
    x: jax.Array,
    k_cache: jax.Array,
    v_cache: jax.Array,
    wq: jax.Array,
    wo: jax.Array,
):
    B, Sq, D = x.shape
    _, Hkv, Sk, Dh = k_cache.shape
    rep = wq.shape[1] // (Hkv * Dh)
    assert B == 8 and Dh == _LANES and Sq % 16 == 0, (B, Dh, Sq)
    assert Sk % (_CHUNKS * _QK_KEYS) == 0, Sk
    bf16 = jnp.bfloat16
    return pl.pallas_call(
        functools.partial(_kernel, rep=rep),
        in_specs=[pl.BlockSpec(memory_space=pl.ANY)] * 5,
        out_specs=pl.BlockSpec(memory_space=pl.ANY),
        out_shape=jax.ShapeDtypeStruct((B, Sq, D), x.dtype),
        scratch_shapes=[
            pltpu.VMEM((B + 1, Sq, D), bf16),
            pltpu.VMEM((2, D, rep * Dh), bf16),
            pltpu.VMEM((3, rep * Dh, D), bf16),
            pltpu.VMEM((B + 1, Sk, Dh), bf16),
            pltpu.VMEM((B + 1, Sk, Dh), bf16),
            pltpu.VMEM((B, Sq, D), x.dtype),
            [pltpu.VMEM((Sq, D), jnp.float32) for _ in range(B)],
            [pltpu.VMEM((rep * Sq, Sk), jnp.float32) for _ in range(2)],
            pltpu.SemaphoreType.DMA((4 + 3 * B + 2 * _COLD * _CHUNKS,)),
            pltpu.SemaphoreType.DMA((B,)),
        ],
        compiler_params=pltpu.CompilerParams(
            vmem_limit_bytes=100 * 1024 * 1024,
            flags={"XLA_TPU_RESCHEDULE_DMA_DONES": True},
            disable_bounds_checks=True,
            disable_semaphore_checks=True,
        ),
    )(x, k_cache, v_cache, wq, wo)
```

```python
import functools

import jax
import jax.numpy as jnp
from jax.experimental import pallas as pl
from jax.experimental.pallas import tpu as pltpu

_LOG2E = 1.4426950408889634
_NN = (((1,), (0,)), ((), ()))
_NT = (((1,), (1,)), ((), ()))
_LANES = 128

_QK_KEYS = 256
_PV_KEYS = 128
_DEPTH = 4
_COLD = 3
_CHUNKS = 4
_FIRST_LOADS = "q0 x0 k0 x1 v0 k1 x2 o0 v1 k2 x3 v2 k3 x4 x5 x6 x7 v3".split()


def _dot(a, b, dims=_NN):
    return jax.lax.dot_general(a, b, dims, preferred_element_type=jnp.float32)


def _lane_tiles(a):
    return [a[:, i:i + _LANES] for i in range(0, a.shape[1], _LANES)]


def _kernel(x_hbm, k_hbm, v_hbm, wq_hbm, wo_hbm, out_hbm,
            x_buf, wq_buf, wo_buf, k_buf, v_buf, out_buf, acc_bufs, s_bufs, in_sems, out_sems,
            *, rep):
    B, Sq, _ = x_hbm.shape
    _, Hkv, Sk, Dh = k_hbm.shape
    G = rep * Dh
    bf16 = jnp.bfloat16
    chunk = Sk // _CHUNKS
    scale = (Dh ** -0.5) * _LOG2E

    sem_base, n_sems = {}, 0
    for name, count in (("wq", 2), ("wo", 2), ("x", B), ("k", B), ("v", B),
                        ("k_chunk", _COLD * _CHUNKS), ("v_chunk", _COLD * _CHUNKS)):
        sem_base[name] = n_sems
        n_sems += count

    def sem(name, i):
        return in_sems.at[sem_base[name] + i]

    kv = {"k": (k_hbm, k_buf), "v": (v_hbm, v_buf)}

    def kv_copy(kind, h, b):
        hbm, buf = kv[kind]
        return pltpu.make_async_copy(hbm.at[b, h], buf.at[b], sem(kind, b))

    def kv_chunk_copy(kind, b, j):
        hbm, buf = kv[kind]
        keys = slice(j * chunk, (j + 1) * chunk)
        return pltpu.make_async_copy(hbm.at[b, 0, keys], buf.at[b, keys],
                                     sem(kind + "_chunk", b * _CHUNKS + j))

    def wq_copy(h):
        cols = pl.ds(pl.multiple_of(h * G, G), G)
        return pltpu.make_async_copy(wq_hbm.at[:, cols], wq_buf.at[h & 1], sem("wq", h & 1))

    def wo_copy(h):
        rows = pl.ds(pl.multiple_of(h * G, G), G)
        return pltpu.make_async_copy(wo_hbm.at[rows, :], wo_buf.at[h & 1], sem("wo", h & 1))

    def x_copy(b):
        return pltpu.make_async_copy(x_hbm.at[b], x_buf.at[b], sem("x", b))

    def out_copy(b):
        return pltpu.make_async_copy(out_buf.at[b], out_hbm.at[b], out_sems.at[b])

    def hold_wait(spare, value):
        spare[...] = value[0:16, 0:_LANES].astype(bf16)

    for token in _FIRST_LOADS:
        kind, i = token[0], int(token[1:])
        if kind in kv and i < _COLD:
            for j in range(_CHUNKS):
                kv_chunk_copy(kind, i, j).start()
        elif kind in kv:
            kv_copy(kind, 0, i).start()
        else:
            {"q": wq_copy, "o": wo_copy, "x": x_copy}[kind](i).start()
    for acc in acc_bufs:
        acc[...] = jnp.zeros_like(acc)

    def prefetch(h, b):
        nb = b + _DEPTH
        if nb < B:
            kv_copy("k", h, nb).start()
            kv_copy("v", h, nb).start()
        else:
            @pl.when(h + 1 < Hkv)
            def _():
                if nb == B:
                    wq_copy(h + 1).start()
                kv_copy("k", h + 1, nb - B).start()
                if nb == B + 1:
                    wo_copy(h + 1).start()
                kv_copy("v", h + 1, nb - B).start()

    def wait_kv(kind, h, b, n, key, after):
        if key == 0 or (n < _COLD and key % chunk == 0):
            if n <= _COLD:
                hold_wait(kv[kind][1].at[B, 0:16, :], after)
            if n < _COLD:
                if key == 0:
                    pl.when(h > 0)(kv_copy(kind, h, b).wait)
                pl.when(h == 0)(kv_chunk_copy(kind, b, key // chunk).wait)
            else:
                kv_copy(kind, h, b).wait()

    def q_proj(h, b, n, after):
        if b == 0:
            wq_copy(h).wait()
        if n < B:
            if after is not None and n <= _COLD:
                hold_wait(x_buf.at[B, 0:16, 0:_LANES], after)
            pl.when(h == 0)(x_copy(b).wait)
        q = _dot(x_buf[b], wq_buf[n // B]) * scale
        stacked = jnp.concatenate([q[:, r * Dh:(r + 1) * Dh] for r in range(rep)], axis=0)
        return stacked.astype(bf16), q

    def scores(h, b, n, q, after):
        per_chunk = chunk // _QK_KEYS
        m, blocks = None, []
        for j, key in enumerate(range(0, Sk, _QK_KEYS)):
            keys = slice(key, key + _QK_KEYS)
            wait_kv("k", h, b, n, key, after if j == 0 else blocks[max(j - per_chunk, 0)])
            s = _dot(q, k_buf[b, keys, :], _NT)
            blocks.append(s)
            s_bufs[b % 2][:, keys] = s
            block_max = functools.reduce(jnp.maximum, _lane_tiles(s))
            m = block_max if m is None else jnp.maximum(m, block_max)
        return jnp.max(m, axis=-1, keepdims=True), blocks[-per_chunk]

    def attend(h, b, n, m, after):
        per_chunk = chunk // _PV_KEYS
        neg_l, o, blocks = None, None, []
        for j, key in enumerate(range(0, Sk, _PV_KEYS)):
            keys = slice(key, key + _PV_KEYS)
            wait_kv("v", h, b, n, key, after if j == 0 else blocks[max(j - per_chunk, 0)])
            p = _lane_tiles(jnp.exp2(s_bufs[b % 2][:, keys] - m))
            for tile in p:
                neg_l = -tile if neg_l is None else neg_l - tile
            p[0] = jnp.maximum(p[0], neg_l)
            part = _dot(jnp.concatenate(p, axis=1).astype(bf16), v_buf[b, keys, :])
            blocks.append(part)
            o = part if o is None else o + part
        neg_l = jnp.minimum(neg_l, jnp.abs(o))
        l = -jnp.sum(neg_l, axis=-1, keepdims=True)
        return o * pl.reciprocal(l, full_range=False), blocks[-per_chunk]

    def out_proj(h, b, n, o, after):
        if b == 0:
            if n == 0:
                hold_wait(wo_buf.at[2, 0:16, 0:_LANES], after)
            wo_copy(h).wait()
        heads = [o[r * Sq:(r + 1) * Sq] for r in range(rep)]
        if n + 1 < 2 * B:
            part = _dot(jnp.concatenate(heads, axis=1).astype(bf16), wo_buf[n // B])
            acc = acc_bufs[b][...] + part
        else:
            acc = acc_bufs[b][...]
            for r in range(rep):
                part = _dot(heads[r].astype(bf16), wo_buf[n // B, r * Dh:(r + 1) * Dh, :])
                acc = acc + part
        acc_bufs[b][...] = acc
        if n >= B:
            out_buf[b] = acc.astype(out_buf.dtype)
            pl.when(h == Hkv - 1)(out_copy(b).start)
        return part

    def head_pair(i, carry):
        steps = [(2 * i + n // B, n % B, n) for n in range(2 * B)]
        q, last = q_proj(*steps[0], None)
        o = None
        for n, step in enumerate(steps):
            m, last = scores(*step, q, last)
            prefetch(*step[:2])
            if n + 1 < len(steps):
                q, last = q_proj(*steps[n + 1], last)
            if n > 0:
                last = out_proj(*steps[n - 1], o, last)
            o, last = attend(*step, m, last)
        out_proj(*steps[-1], o, None)
        return carry

    jax.lax.fori_loop(0, Hkv // 2, head_pair, 0)
    for b in range(B):
        out_copy(b).wait()


@jax.jit
def pallas_standalone__gqa_block_cached__near_ridge_kernel(
    x: jax.Array,
    k_cache: jax.Array,
    v_cache: jax.Array,
    wq: jax.Array,
    wo: jax.Array,
):
    B, Sq, D = x.shape
    _, Hkv, Sk, Dh = k_cache.shape
    rep = wq.shape[1] // (Hkv * Dh)
    assert B == 8 and Hkv % 2 == 0 and Dh == _LANES and Sq % 16 == 0, (B, Hkv, Dh, Sq)
    assert Sk % (_CHUNKS * _QK_KEYS) == 0, Sk
    bf16 = jnp.bfloat16
    return pl.pallas_call(
        functools.partial(_kernel, rep=rep),
        in_specs=[pl.BlockSpec(memory_space=pl.ANY)] * 5,
        out_specs=pl.BlockSpec(memory_space=pl.ANY),
        out_shape=jax.ShapeDtypeStruct((B, Sq, D), x.dtype),
        scratch_shapes=[
            pltpu.VMEM((B + 1, Sq, D), bf16),
            pltpu.VMEM((2, D, rep * Dh), bf16),
            pltpu.VMEM((3, rep * Dh, D), bf16),
            pltpu.VMEM((B + 1, Sk, Dh), bf16),
            pltpu.VMEM((B + 1, Sk, Dh), bf16),
            pltpu.VMEM((B, Sq, D), x.dtype),
            [pltpu.VMEM((Sq, D), jnp.float32) for _ in range(B)],
            [pltpu.VMEM((rep * Sq, Sk), jnp.float32) for _ in range(2)],
            pltpu.SemaphoreType.DMA((4 + 3 * B + 2 * _COLD * _CHUNKS,)),
            pltpu.SemaphoreType.DMA((B,)),
        ],
        compiler_params=pltpu.CompilerParams(
            vmem_limit_bytes=100 * 1024 * 1024,
            flags={"XLA_TPU_RESCHEDULE_DMA_DONES": True},
            disable_bounds_checks=True,
            disable_semaphore_checks=True,
        ),
    )(x, k_cache, v_cache, wq, wo)
```
